```python
import os as _os
_os.environ.setdefault("JAX_PLATFORMS", "cpu")
import jax
import jax.numpy as jnp

def _softmax(x, axis=-1):
    return jax.nn.softmax(x, axis=axis)
def _gelu(x):
    return jax.nn.gelu(x, approximate=True)
def _silu(x):
    return jax.nn.silu(x)
def _sigmoid(x):
    return jax.nn.sigmoid(x)
def _layernorm(x, axis=-1, eps=1e-5):
    m = jnp.mean(x, axis=axis, keepdims=True)
    v = jnp.var(x, axis=axis, keepdims=True)
    return (x - m) / jnp.sqrt(v + eps)
def _scatter_add(tgt, idx, src, axis=0):
    return tgt.at[idx].add(src)
def _segment_sum(src, seg, n):
    return jax.ops.segment_sum(src, seg, n)
class _Rng:
    def __init__(self, key):
        self._k = key
    def _next(self):
        self._k, sub = jax.random.split(self._k)
        return sub
    def normal(self, shape):
        return jax.random.normal(self._next(), shape, dtype=jnp.bfloat16)
    def randint(self, lo, hi, shape):
        return jax.random.randint(self._next(), shape, lo, hi, dtype=jnp.int32)
    def uniform(self, shape, lo=0.0, hi=1.0):
        return jax.random.uniform(self._next(), shape, jnp.bfloat16, lo, hi)
    def permutation(self, n):
        return jax.random.permutation(self._next(), n)


kernel_name = 'concat_heads__linear_kernel_hedgehog__ssm_conv_s5__prompt'

def setup_inputs():
    _rng = _Rng(jax.random.key(int.from_bytes(__import__("os").urandom(4), "little")))
    _w = (lambda a: (lambda t: t.astype(jnp.bfloat16) if jnp.issubdtype(t.dtype, jnp.floating) else t)(jnp.asarray(a)))
    def _A_setup():
        B, S, D, H = 1, 2048, 640, 32
        Dh = D // H
        return {
            "x": _w((lambda *s: _rng.normal(s) * 0.4)(B, S, D)),
            "wqkv": _w((lambda *s: _rng.normal(s) * 0.4)(D, 3 * D)),
            "w_phi": _w((lambda *s: _rng.normal(s) * 0.4)(H, Dh, Dh) * (Dh ** -0.5)),
            "wo": _w((lambda *s: _rng.normal(s) * 0.05)(D, D)),
        }
    _A_in = _A_setup()

    def _B_setup():
        B, S, D = 1, 2048, 640
        P = D
        Lambda_re = -0.5 * jnp.exp((lambda *s: _rng.normal(s) * 0.8)(P))
        Lambda_im = (lambda *s: _rng.normal(s) * 0.8)(P) * 1.0
        B_re = (lambda *s: _rng.normal(s) * 0.8)(P, D) * (D ** -0.5)
        B_im = (lambda *s: _rng.normal(s) * 0.8)(P, D) * (D ** -0.5)
        C_re = (lambda *s: _rng.normal(s) * 0.8)(D, P) * (P ** -0.5)
        C_im = (lambda *s: _rng.normal(s) * 0.8)(D, P) * (P ** -0.5)
        log_dt = (lambda *s: _rng.normal(s) * 0.8)(P) * 0.3 - 2.0
        Dskip = (lambda *s: _rng.normal(s) * 0.8)(D)
        return {
            "x": _w((lambda *s: _rng.normal(s) * 0.05)(B, S, D)),
            "Lambda_re": _w(Lambda_re),
            "Lambda_im": _w(Lambda_im),
            "B_re": _w(B_re),
            "B_im": _w(B_im),
            "C_re": _w(C_re),
            "C_im": _w(C_im),
            "log_dt": _w(log_dt),
            "Dskip": _w(Dskip),
        }
    _B_in = _B_setup()

    return {
        "A_x": _A_in["x"],
        "A_wqkv": _A_in["wqkv"],
        "A_w_phi": _A_in["w_phi"],
        "A_wo": _A_in["wo"],
        "B_x": _B_in["x"],
        "B_Lambda_re": _B_in["Lambda_re"],
        "B_Lambda_im": _B_in["Lambda_im"],
        "B_B_re": _B_in["B_re"],
        "B_B_im": _B_in["B_im"],
        "B_C_re": _B_in["C_re"],
        "B_C_im": _B_in["C_im"],
        "B_log_dt": _B_in["log_dt"],
        "B_Dskip": _B_in["Dskip"],
    }

def reference(A_x, A_wqkv, A_w_phi, A_wo, B_x, B_Lambda_re, B_Lambda_im, B_B_re, B_B_im, B_C_re, B_C_im, B_log_dt, B_Dskip):
    def _A_ref(x, wqkv, w_phi, wo):
        B, S, D = x.shape
        H = 32; Dh = D // H
        qkv = (lambda x, *d: x.transpose(*d))((x @ wqkv).reshape(B, S, 3, H, Dh), 2, 0, 3, 1, 4)
        q, k, v = qkv[0], qkv[1], qkv[2]
        pq = jnp.einsum("bhsd,hdf->bhsf", q, w_phi)
        pk = jnp.einsum("bhsd,hdf->bhsf", k, w_phi)
        phi_q = jnp.concatenate([_softmax(pq, axis=-1), _softmax(-pq, axis=-1)], axis=-1)
        phi_k = jnp.concatenate([_softmax(pk, axis=-1), _softmax(-pk, axis=-1)], axis=-1)
        kv = jnp.einsum("bhsf,bhsd->bhfd", phi_k, v)
        z  = jnp.einsum("bhsf->bhf", phi_k)
        num = jnp.einsum("bhqf,bhfd->bhqd", phi_q, kv)
        den = jnp.einsum("bhqf,bhf->bhq", phi_q, z)[..., None] + 1e-6
        o = num / den
        return (lambda x, *d: x.transpose(*d))(o, 0, 2, 1, 3).reshape(B, S, D) @ wo

    def _B_ref(x, Lambda_re, Lambda_im, B_re, B_im, C_re, C_im, log_dt, Dskip):
        Bsz, L, H = x.shape
        Lam = Lambda_re + 1j * Lambda_im
        Bmat = B_re + 1j * B_im
        Cmat = C_re + 1j * C_im
        dt = jnp.exp(log_dt)
        Lam_bar = jnp.exp(dt * Lam)
        B_bar = ((Lam_bar - 1.0) / Lam)[:, None] * Bmat
        Bu = jnp.einsum("bld,pd->blp", x + 0j, B_bar)
        h = jnp.zeros_like(Bu[:, 0, :])
        hs = []
        for t in range(L):
            h = Lam_bar[None, :] * h + Bu[:, t, :]
            hs.append(h)
        hseq = jnp.stack(hs, 1)
        y = 2.0 * jnp.einsum("blp,dp->bld", hseq, Cmat).real + x * Dskip[None, None, :]
        return y

    a = _A_ref(A_x, A_wqkv, A_w_phi, A_wo)
    b = _B_ref(B_x, B_Lambda_re, B_Lambda_im, B_B_re, B_B_im, B_C_re, B_C_im, B_log_dt, B_Dskip)
    return jnp.concatenate([a, b], axis=-1)
```

```python
import jax
import jax.numpy as jnp
from jax import lax
import jax.experimental.pallas as pl
import jax.experimental.pallas.tpu as pltpu

S, D, H, DH = 2048, 640, 32, 20
NS = 8
SR = 80
NJ = S // 128
NSEG, SEG = 8, 256
JB = 32
NB = SEG // JB
PITCH = JB + 4
BROWS = NSEG * PITCH
KT = D // 128
F32, BF16 = jnp.float32, jnp.bfloat16
NT = (((1,), (1,)), ((), ()))
NN = (((1,), (0,)), ((), ()))
TN = (((0,), (0,)), ((), ()))
TT = (((0,), (1,)), ((), ()))
LOG2E = 1.4426950408889634
T = 512
NC = S // T
TQ = 512
OCUT = tuple(range(17))


def _dot(a, b, dn):
    return lax.dot_general(a, b, dn, preferred_element_type=F32)


def _lanes(xs):
    return jnp.concatenate(xs, axis=1)


def _mix(main, *fill):
    main = list(main)
    fill = [list(f) for f in fill]
    n = len(main)
    done = [0] * len(fill)
    for i, m in enumerate(main):
        m()
        for k, f in enumerate(fill):
            upto = (len(f) * (i + 1) + n - 1) // n
            while done[k] < upto:
                f[done[k]]()
                done[k] += 1


def _kernel(ax_h, wqkv_h, wphi_h, wo_h, bx_h, lre_h, lim_h, bre_h, bim_h, cre_h, cim_h,
            ldt_h, dsk_h, out_h,
            ax, wqkv, wphi, wo, bx, lre_v, lim_v, ldt_v, dsk_v, bmat, cmat,
            cw, bu0, bu1, hbuf, yst, ob, bdb, wq, wkv, phk, vts, zacc, kvm, ots, oa,
            isem, osem):
    nsem = [0]

    def cp(src, dst):
        nsem[0] += 1
        return pltpu.make_async_copy(src, dst, isem.at[nsem[0] - 1])
    d_vec = [cp(lre_h, lre_v), cp(lim_h, lim_v), cp(ldt_h, ldt_v), cp(dsk_h, dsk_v)]
    d_b = [cp(bre_h, bmat.at[0]), cp(bim_h, bmat.at[1])]
    d_c = [cp(cre_h, cmat.at[0]), cp(cim_h, cmat.at[1])]
    d_wphi, d_wqkv, d_wo = cp(wphi_h, wphi), cp(wqkv_h, wqkv), cp(wo_h, wo)
    d_bx = [cp(bx_h.at[:, pl.ds(b * JB, JB), :], bx.at[b]) for b in range(NB)]
    d_ax = [cp(ax_h.at[pl.ds(c * 512, 512), :], ax.at[pl.ds(c * 512, 512), :]) for c in range(4)]

    grp = [d_b[0:1] + d_bx[0:2], d_b[1:2] + d_bx[2:3] + d_vec, d_bx[3:8] + d_c,
           [d_wphi, d_wqkv], d_ax + [d_wo]]
    for g_ in grp:
        for d in g_:
            d.start()

    def need(i):
        for d in grp[i]:
            d.wait()

    st = {}
    bu = (bu0, bu1)

    def discretise():
        lre = lre_v[...].astype(F32).reshape(1, D)
        lim = lim_v[...].astype(F32).reshape(1, D)
        dt = jnp.exp(ldt_v[...].astype(F32).reshape(1, D)).astype(BF16).astype(F32)
        st['dsk'] = dsk_v[...].astype(F32).reshape(1, D)
        are, aim = dt * lre, dt * lim
        mag = jnp.exp(are)
        lbr, lbi = mag * jnp.cos(aim), mag * jnp.sin(aim)
        inv = 1.0 / (lre * lre + lim * lim)
        nr, ni = lbr - 1.0, lbi
        st['cr2'] = 2.0 * (nr * lre + ni * lim) * inv
        st['ci2'] = 2.0 * (ni * lre - nr * lim) * inv
        st['lbr'], st['lbi'] = lbr, lbi
        lr8 = jnp.broadcast_to(lbr, (8, D))
        li8 = jnp.broadcast_to(lbi, (8, D))
        st['lrs'] = [lr8[:, t * 128:(t + 1) * 128] for t in range(KT)]
        st['lis'] = [li8[:, t * 128:(t + 1) * 128] for t in range(KT)]
        st['h'] = [jnp.zeros((8, 128), F32) for _ in range(2 * KT)]

    def scan_step(b, jj):
        h, lrs, lis = st['h'], st['lrs'], st['lis']
        out = []
        for t in range(KT):
            hr, hi = h[2 * t], h[2 * t + 1]
            idx = pl.ds((b // 2) * BROWS + jj, NSEG, stride=PITCH)
            out.append(lrs[t] * hr - lis[t] * hi + bu[b % 2][t, idx, :])
            out.append(lrs[t] * hi + lis[t] * hr + bu[b % 2][KT + t, idx, :])
        st['h'] = out
        return out

    def bu_dots(b):
        def one(ri):
            def f():
                u = _dot(bx[b].reshape(NSEG * JB, D), bmat[ri], NT)
                for t in range(KT):
                    for s in range(NSEG):
                        r0 = (b // 2) * BROWS + s * PITCH
                        bu[b % 2][ri * KT + t, r0:r0 + JB, :] = u[s * JB:(s + 1) * JB, t * 128:(t + 1) * 128]
            return f
        return [one(ri) for ri in range(2)]

    def scan1(b):
        return [(lambda jj=jj: scan_step(b, jj)) for jj in range(JB)]

    def make_cw():
        def one(t, r):
            def f():
                sl, rs = slice(t * 128, (t + 1) * 128), slice(r * 128, (r + 1) * 128)
                c_re, c_im = cmat[0, rs, sl].astype(F32), cmat[1, rs, sl].astype(F32)
                cr2, ci2 = st['cr2'][:, sl], st['ci2'][:, sl]
                cw[t, rs, :] = (c_re * cr2 - c_im * ci2).astype(BF16)
                cw[KT + t, rs, :] = (-(c_re * ci2 + c_im * cr2)).astype(BF16)
            return f
        return [one(t, r) for t in range(KT) for r in range(KT)]

    def carry():
        h = st['h']
        p_r, p_i = st['lbr'], st['lbi']
        for _ in range(8):
            p_r, p_i = p_r * p_r - p_i * p_i, 2.0 * p_r * p_i
        e_r = _lanes([h[2 * t] for t in range(KT)])
        e_i = _lanes([h[2 * t + 1] for t in range(KT)])
        car_r, car_i = [jnp.zeros((1, D), F32)], [jnp.zeros((1, D), F32)]
        for s in range(NSEG - 1):
            a_r, a_i = car_r[-1], car_i[-1]
            car_r.append(e_r[s:s + 1] + p_r * a_r - p_i * a_i)
            car_i.append(e_i[s:s + 1] + p_r * a_i + p_i * a_r)
        c_r = jnp.concatenate(car_r, axis=0)
        c_i = jnp.concatenate(car_i, axis=0)
        h = []
        for t in range(KT):
            h += [c_r[:, t * 128:(t + 1) * 128], c_i[:, t * 128:(t + 1) * 128]]
        st['h'] = h

    def scan2(b):
        def one(jj):
            def f():
                h0 = scan_step(b, jj)
                h1 = scan_step(b, jj + 1)
                for t in range(KT):
                    for ri in range(2):
                        v = jnp.concatenate([h0[2 * t + ri], h1[2 * t + ri]], axis=0).astype(BF16)
                        hbuf[b, ri * KT + t, jj * 8:jj * 8 + 16, :] = v
            return f
        return [one(jj) for jj in range(0, JB, 2)]

    def y_dots(b):
        def f():
            hb = _lanes([hbuf[b, k] for k in range(2 * KT)])
            wt = _lanes([cw[k] for k in range(2 * KT)])
            y = _dot(hb, wt, NT)
            for t in range(KT):
                for jj in range(JB):
                    yst[b, t, pl.ds(jj, NSEG, stride=PITCH), :] = y[jj * 8:jj * 8 + 8, t * 128:(t + 1) * 128]
        return [f]

    def ob_copy(b):
        return pltpu.make_async_copy(ob.at[b], out_h.at[:, pl.ds(b * JB, JB), pl.ds(D, D)], osem.at[b])

    def finalize(b):
        def one(s):
            def f():
                xs = bx[b, s].astype(F32) * st['dsk']
                for t in range(KT):
                    ob[b, s, :, t * 128:(t + 1) * 128] = (
                        yst[b, t, s * PITCH:s * PITCH + JB, :] + xs[:, t * 128:(t + 1) * 128])
            return f
        return [one(s) for s in range(NSEG)]

    def make_bd():
        def one(d):
            def f():
                fi = lax.broadcasted_iota(jnp.int32, (DH, 128), 0)
                mi = lax.broadcasted_iota(jnp.int32, (DH, 128), 1)
                rmat = ((mi >> 2) == fi).astype(BF16)
                hi_ = lax.broadcasted_iota(jnp.int32, (H, 128), 0)
                mj = lax.broadcasted_iota(jnp.int32, (H, 128), 1)
                a = jnp.where((hi_ & 3) == (mj & 3), _dot(wphi[d], rmat, TN), 0.0)
                for hb in range(H // 8):
                    bdb[pl.ds(hb * 8 * DH + d, 8, stride=DH), :] = a[hb * 8:hb * 8 + 8, :]
            return f
        return [one(d) for d in range(DH)]

    def make_wvt():
        def one(k):
            def f():
                wt = wqkv[k * 128:(k + 1) * 128, 2 * D:3 * D].T
                for g in range(NS // 2):
                    wkv[g, k, 2 * SR:4 * SR, :] = wt[g * 2 * SR:(g + 1) * 2 * SR, :]
            return f
        return [one(k) for k in range(KT)]

    def fold(w):
        def one(sb):
            def f():
                a0 = (sb * SR) // 128 * 128
                a1 = -(-(sb + 1) * SR // 128) * 128
                kidx = lax.broadcasted_iota(jnp.int32, (a1 - a0, SR), 0) + a0
                win = jnp.where((kidx >= sb * SR) & (kidx < (sb + 1) * SR), bdb[a0:a1, 0:SR], 0.0).astype(BF16)
                wp = (_dot(win, wqkv[:, w * D + a0:w * D + a1], TT) * LOG2E).astype(BF16)
                dst = wq if w == 0 else wkv
                r0 = (sb % 2) * SR
                for k in range(KT):
                    dst[sb // 2, k, r0:r0 + SR, :] = wp[:, k * 128:(k + 1) * 128]
            return f
        return [one(sb) for sb in range(NS)]

    need(0)
    bu_dots(0)[0]()
    bu_dots(1)[0]()
    need(1)
    discretise()
    bu_dots(0)[1]()
    bu_dots(1)[1]()
    _mix(bu_dots(2), scan1(0) + scan1(1))
    need(2)
    for b in range(3, NB):
        extra = []
        if b == 3:
            extra = make_cw()
        if b == 6:
            need(3)
            extra = make_bd() + make_wvt()
        _mix(bu_dots(b), scan1(b - 1), extra)

    _mix(fold(1), scan1(NB - 1) + [carry])
    _mix(fold(0), scan2(0))

    for b in range(NB):
        _mix(y_dots(b), scan2(b + 1) if b + 1 < NB else [], finalize(b - 1) if b >= 1 else [])
    for f in finalize(NB - 1):
        f()

    need(4)
    for b in range(NB):
        ob_copy(b).start()
    def half(x, op):
        return op(x, pltpu.roll(x, 4, 0))

    def feats(p):
        sl = [p[i * 8:i * 8 + 8, :] for i in range(SR // 8)]
        mx, mn = sl[0], sl[0]
        for a in sl[1:]:
            mx = jnp.maximum(mx, a)
            mn = jnp.minimum(mn, a)
        mx, mn = half(mx, jnp.maximum), half(mn, jnp.minimum)
        e1 = [jnp.exp2(a - mx) for a in sl]
        e2 = [jnp.exp2(mn - a) for a in sl]
        r1 = 1.0 / half(sum(e1[1:], e1[0]), jnp.add)
        r2 = 1.0 / half(sum(e2[1:], e2[0]), jnp.add)
        return e1, e2, r1, r2

    for g in range(NS // 2):
        for c in range(NC):
            p = _dot(_lanes([wkv[g, k] for k in range(KT)]), ax[c * T:(c + 1) * T, :], NT)
            for u in range(2):
                sb = 2 * g + u
                e1, e2, r1, r2 = feats(p[u * SR:(u + 1) * SR])
                ph = jnp.concatenate([a * r1 for a in e1] + [a * r2 for a in e2], axis=0)
                zs = ph[:, 0:128]
                for l in range(1, T // 128):
                    zs = zs + ph[:, l * 128:(l + 1) * 128]
                if c == 0:
                    zacc[sb] = zs
                else:
                    zacc[sb] += zs
                phb = ph.astype(BF16)
                vb = p[(2 + u) * SR:(3 + u) * SR].astype(BF16)
                for l in range(T // 128):
                    phk[sb, c * (T // 128) + l] = phb[:, l * 128:(l + 1) * 128]
                    vts[sb, c * (T // 128) + l] = vb[:, l * 128:(l + 1) * 128]
        for u in range(2):
            sb = 2 * g + u
            kv = _dot(_lanes([vts[sb, j] for j in range(NJ)]), _lanes([phk[sb, j] for j in range(NJ)]), NT)
            ri = lax.broadcasted_iota(jnp.int32, (SR, 2 * SR), 0)
            ci = lax.broadcasted_iota(jnp.int32, (SR, 2 * SR), 1)
            kmask = jnp.floor((ri.astype(F32) + 0.5) * (1.0 / DH)) == (ci & 3).astype(F32)
            kvm[sb] = jnp.where(kmask, kv, 0.0).astype(BF16)
            z = jnp.sum(zacc[sb], axis=1, keepdims=True)
            zacc[sb] = jnp.broadcast_to(z, (2 * SR, 128))

    def oa_copy(j):
        return pltpu.make_async_copy(oa.at[j], out_h.at[j // 2, pl.ds((j % 2) * 128, 128), pl.ds(0, D)],
                                     osem.at[NB + j])

    for c in range(S // TQ):
        for g in range(NS // 2):
            p = _dot(_lanes([wq[g, k] for k in range(KT)]), ax[c * TQ:(c + 1) * TQ, :], NT)
            for u in range(2):
                sb = 2 * g + u
                e1, e2, r1, r2 = feats(p[u * SR:(u + 1) * SR])

                def wsum(e, off):
                    acc = None
                    for i in range(SR // 8):
                        z = zacc[sb, off + i * 8:off + i * 8 + 8, :]
                        z = _lanes([z] * (TQ // 128))
                        acc = e[i] * z if acc is None else acc + e[i] * z
                    return acc
                rden = 1.0 / (half(wsum(e1, 0) * r1 + wsum(e2, SR) * r2, jnp.add) + 1e-6)
                s1, s2 = r1 * rden, r2 * rden
                ph = jnp.concatenate([a * s1 for a in e1] + [a * s2 for a in e2], axis=0).astype(BF16)
                ots[c, sb * SR:(sb + 1) * SR, :] = _dot(kvm[sb], ph, NN).astype(BF16)
        last = c == S // TQ - 1
        mt = 128 if last else TQ
        ot_t = ots[c].T
        for m0 in range(0, TQ, mt):
            o = _dot(ot_t[m0:m0 + mt], wo[...], NN)
            for l in range(mt // 128):
                j = (c * TQ + m0) // 128 + l
                oa[j] = o[l * 128:(l + 1) * 128, :]
                if j + 1 in OCUT:
                    for jj in range(OCUT[OCUT.index(j + 1) - 1], j + 1):
                        oa_copy(jj).start()

    for b in range(NB):
        ob_copy(b).wait()
    for j in range(NJ):
        oa_copy(j).wait()


@jax.jit
def pallas_concat_heads__linear_kernel_hedgehog__ssm_conv_s5__prompt_kernel(
    A_x, A_wqkv, A_w_phi, A_wo, B_x, B_Lambda_re, B_Lambda_im, B_B_re, B_B_im,
    B_C_re, B_C_im, B_log_dt, B_Dskip,
):
    vm = pltpu.VMEM
    hbm = pl.BlockSpec(memory_space=pltpu.HBM)
    out = pl.pallas_call(
        _kernel,
        out_shape=jax.ShapeDtypeStruct((NSEG, SEG, 2 * D), F32),
        in_specs=[hbm] * 13,
        out_specs=hbm,
        scratch_shapes=[
            vm((S, D), BF16), vm((D, 3 * D), BF16), vm((DH, DH, H), BF16), vm((D, D), BF16),
            vm((NB, NSEG, JB, D), BF16),
            vm((D,), BF16), vm((D,), BF16), vm((D,), BF16), vm((D,), BF16),
            vm((2, D, D), BF16), vm((2, D, D), BF16),
            vm((2 * KT, D, 128), BF16), vm((2 * KT, NB // 2 * BROWS, 128), F32), vm((2 * KT, NB // 2 * BROWS, 128), F32),
            vm((NB, 2 * KT, NSEG * JB, 128), BF16), vm((NB, KT, BROWS, 128), F32),
            vm((NB, NSEG, JB, D), F32),
            vm((D, 128), F32), vm((NS // 2, KT, 2 * SR, 128), BF16), vm((NS // 2, KT, 4 * SR, 128), BF16),
            vm((NS, NJ, 2 * SR, 128), BF16), vm((NS, NJ, SR, 128), BF16),
            vm((NS, 2 * SR, 128), F32), vm((NS, SR, 2 * SR), BF16),
            vm((S // TQ, D, TQ), BF16), vm((NJ, 128, D), F32),
            pltpu.SemaphoreType.DMA((40,)), pltpu.SemaphoreType.DMA((NB + NJ,)),
        ],
        compiler_params=pltpu.CompilerParams(vmem_limit_bytes=100 * 1024 * 1024),
    )(A_x.reshape(S, D), A_wqkv, A_w_phi.transpose(1, 2, 0), A_wo, B_x.reshape(NSEG, SEG, D),
      B_Lambda_re, B_Lambda_im, B_B_re, B_B_im, B_C_re, B_C_im, B_log_dt, B_Dskip)
    return out.reshape(1, S, 2 * D)
```
